```python
import jax
import jax.numpy as jnp

def _softmax(x, axis=-1):
    return jax.nn.softmax(x, axis=axis)

def _gelu(x):
    return jax.nn.gelu(x, approximate=True)

def _silu(x):
    return jax.nn.silu(x)

def _sigmoid(x):
    return jax.nn.sigmoid(x)

def _layernorm(x, axis=-1, eps=1e-05):
    m = jnp.mean(x, axis=axis, keepdims=True)
    v = jnp.var(x, axis=axis, keepdims=True)
    return (x - m) / jnp.sqrt(v + eps)

def _scatter_add(tgt, idx, src, axis=0):
    return tgt.at[idx].add(src)

def _segment_sum(src, seg, n):
    return jax.ops.segment_sum(src, seg, n)

class _Rng:

    def __init__(self, key):
        self._k = key

    def _next(self):
        self._k, sub = jax.random.split(self._k)
        return sub

    def normal(self, shape):
        return jax.random.normal(self._next(), shape, dtype=jnp.bfloat16)

    def randint(self, lo, hi, shape):
        return jax.random.randint(self._next(), shape, lo, hi, dtype=jnp.int32)

    def uniform(self, shape, lo=0.0, hi=1.0):
        return jax.random.uniform(self._next(), shape, jnp.bfloat16, lo, hi)

    def permutation(self, n):
        return jax.random.permutation(self._next(), n)
kernel_name = 'adaLN_cond__sliding_block_cached__moe_arch_mod__prompt'

def setup_inputs():
    _rng = _Rng(jax.random.key(int.from_bytes(__import__("os").urandom(4), "little")))
    _w = lambda a: (lambda t: t.astype(jnp.bfloat16) if jnp.issubdtype(t.dtype, jnp.floating) else t)(jnp.asarray(a))

    def _A_setup():
        B, Sq, D = (1, 2048, 1024)
        Hq, Hkv, Sk, Dh = (32, 4, 2048, 128)
        assert Hq % Hkv == 0, (Hq, Hkv)
        return {'x': _w((lambda *s: _rng.normal(s) * 0.05)(B, Sq, D)), 'k_cache': _w((lambda *s: _rng.normal(s) * 0.05)(B, Hkv, Sk, Dh)), 'v_cache': _w((lambda *s: _rng.normal(s) * 0.05)(B, Hkv, Sk, Dh)), 'wq': _w((lambda *s: _rng.normal(s) * 0.05)(D, Hq * Dh) * D ** (-0.5)), 'wo': _w((lambda *s: _rng.normal(s) * 0.05)(Hq * Dh, D) * (Hq * Dh) ** (-0.5))}
    _A_in = _A_setup()

    def _B_setup():
        B, S, D, F, C = (1, 2048, 1024, 3584, 1)
        return {'x': _w((lambda *s: _rng.normal(s) * 0.05)(B, S, D)), 'w_r': _w((lambda *s: _rng.normal(s) * 0.05)(D)), 'w_gate': _w((lambda *s: _rng.normal(s) * 0.05)(D, F)), 'w_up': _w((lambda *s: _rng.normal(s) * 0.05)(D, F)), 'w_down': _w((lambda *s: _rng.normal(s) * 0.05)(F, D))}
    _B_in = _B_setup()
    return {'A_x': _A_in['x'], 'A_k_cache': _A_in['k_cache'], 'A_v_cache': _A_in['v_cache'], 'A_wq': _A_in['wq'], 'A_wo': _A_in['wo'], 'B_x': _B_in['x'], 'B_w_r': _B_in['w_r'], 'B_w_gate': _B_in['w_gate'], 'B_w_up': _B_in['w_up'], 'B_w_down': _B_in['w_down'], 'c': _w((lambda *s: _rng.normal(s) * 0.05)(1, 1024)), 'w_mod': _w((lambda *s: _rng.normal(s) * 0.05)(1024, 6 * 1024) * 1024 ** (-0.5))}

def reference(A_x, A_k_cache, A_v_cache, A_wq, A_wo, B_x, B_w_r, B_w_gate, B_w_up, B_w_down, c, w_mod):

    def _A_ref(x, k_cache, v_cache, wq, wo):
        B, Sq, D = x.shape
        Hq, Dh = (32, 128)
        Hkv, Sk = (k_cache.shape[1], k_cache.shape[2])
        W = min(4096, max(256, Sk // 4))
        rep = Hq // Hkv
        q = (lambda x, *d: x.transpose(*d))((x @ wq).reshape(B, Sq, Hq, Dh), 0, 2, 1, 3)
        k = jnp.repeat(k_cache[:, :, Sk - W:, :], rep, axis=1)
        v = jnp.repeat(v_cache[:, :, Sk - W:, :], rep, axis=1)
        scores = jnp.einsum('bhqd,bhkd->bhqk', q, k) * Dh ** (-0.5)
        p = _softmax(scores, axis=-1)
        o = jnp.einsum('bhqk,bhkd->bhqd', p, v)
        return (lambda x, *d: x.transpose(*d))(o, 0, 2, 1, 3).reshape(B, Sq, Hq * Dh) @ wo

    def _B_ref(x, w_r, w_gate, w_up, w_down):
        B, S, D = x.shape
        C = 1
        r = x @ w_r
        idx = jnp.argsort(-r, axis=-1)[:, :C]
        idx_e = jnp.repeat(idx.reshape(B, C, 1), D, axis=2)
        x_sel = jnp.take_along_axis(x, idx_e, axis=1)
        g = _silu(x_sel @ w_gate)
        u = x_sel @ w_up
        y = g * u @ w_down
        r_sel = _sigmoid(jnp.take_along_axis(r, idx, axis=1))
        y = y * r_sel.reshape(B, C, 1)
        b_off = (jnp.arange(B) * S).reshape(B, 1)
        flat_idx = (idx + b_off).reshape(B * C)
        zero = (x * 0.0).reshape(B * S, D)
        upd = _scatter_add(zero, flat_idx, y.reshape(B * C, D), axis=0)
        return x + upd.reshape(B, S, D)
    x = A_x
    mod = (_silu(c) @ w_mod).reshape(c.shape[0], 6, 1, -1)
    sa, ca, ga, sb, cb, gb = (mod[:, 0].copy(), mod[:, 1].copy(), mod[:, 2].copy(), mod[:, 3].copy(), mod[:, 4].copy(), mod[:, 5].copy())
    h = _layernorm(x, axis=-1) * (1 + ca) + sa
    x = x + ga * _A_ref(h, A_k_cache, A_v_cache, A_wq, A_wo)
    h = _layernorm(x, axis=-1) * (1 + cb) + sb
    x = x + gb * _B_ref(h, B_w_r, B_w_gate, B_w_up, B_w_down)
    return x
```

```python
import math

import jax
import jax.numpy as jnp
import jax.experimental.pallas as pl
import jax.experimental.pallas.tpu as pltpu

_S = 2048
_D = 1024
_HQ = 32
_HKV = 4
_DH = 128
_SK = 2048
_W = 512
_F = 3584
_REP = _HQ // _HKV
_GW = _REP * _DH
_TM = 512
_NT = _S // _TM
_EPS = 1e-5
_QSCALE = (_DH ** -0.5) * math.log2(math.e)

_BF = jnp.bfloat16
_F32 = jnp.float32


def _layernorm(x):
    m = jnp.mean(x, axis=-1, keepdims=True)
    xc = x - m
    v = jnp.mean(xc * xc, axis=-1, keepdims=True)
    return xc * jax.lax.rsqrt(v + _EPS)


def _silu(x):
    return x * jax.nn.sigmoid(x)


def _kernel(
    x_hbm, k_hbm, v_hbm, wq_hbm, wo_hbm, wr_ref, wg_hbm, wu_hbm, wd_hbm, c_ref,
    wmod_hbm,
    out_hbm,
    x_vmem, out_vmem, h2_vmem, k_vmem, kt_vmem, v_vmem, wq_vmem, wo_vmem,
    wmod_vmem, wg_vmem, wu_vmem, wd_vmem, h_scr, o_scr, acc_scr, mod_scr,
    best_smem, bidx_smem,
    x_sem, out_sem, kv_sem, wq_sem, wo_sem, wmod_sem, ffn_sem, fix_sem,
):
    def x_copy(t):
        return pltpu.make_async_copy(
            x_hbm.at[0, pl.ds(t * _TM, _TM), :],
            x_vmem.at[pl.ds(t * _TM, _TM), :],
            x_sem.at[t])

    def out_copy(t):
        return pltpu.make_async_copy(
            out_vmem.at[pl.ds(t * _TM, _TM), :],
            out_hbm.at[0, pl.ds(t * _TM, _TM), :],
            out_sem.at[t])

    def wmod_copy(j):
        return pltpu.make_async_copy(
            wmod_hbm.at[:, pl.ds(j * _D, _D)],
            wmod_vmem.at[:, pl.ds(j * _D, _D)],
            wmod_sem.at[j])

    def wq_copy(g):
        return pltpu.make_async_copy(
            wq_hbm.at[:, pl.ds(g * _GW, _GW)],
            wq_vmem.at[:, pl.ds(g * _GW, _GW)],
            wq_sem.at[g])

    def wo_copy(g):
        return pltpu.make_async_copy(
            wo_hbm.at[pl.ds(g * _GW, _GW), :],
            wo_vmem.at[pl.ds(g * _GW, _GW), :],
            wo_sem.at[g])

    k_copy = pltpu.make_async_copy(
        k_hbm.at[0, :, pl.ds(_SK - _W, _W), :], k_vmem, kv_sem.at[0])
    v_copy = pltpu.make_async_copy(
        v_hbm.at[0, :, pl.ds(_SK - _W, _W), :], v_vmem, kv_sem.at[1])
    wg_copy = pltpu.make_async_copy(wg_hbm, wg_vmem, ffn_sem.at[0])
    wu_copy = pltpu.make_async_copy(wu_hbm, wu_vmem, ffn_sem.at[1])
    wd_copy = pltpu.make_async_copy(wd_hbm, wd_vmem, ffn_sem.at[2])

    wmod_copy(0).start()
    wmod_copy(1).start()
    x_copy(0).start()
    wq_copy(0).start()
    k_copy.start()
    v_copy.start()

    c = c_ref[...].astype(_F32)
    sc = jnp.broadcast_to(_silu(c), (16, _D)).astype(_BF)

    def mod_chunk(j):
        wmod_copy(j).wait()
        r = jnp.dot(sc, wmod_vmem[:, j * _D:(j + 1) * _D],
                    preferred_element_type=_F32)
        mod_scr[j:j + 1, :] = r[0:1, :]

    mod_chunk(0)
    mod_chunk(1)
    for g in range(1, _HKV):
        wq_copy(g).start()
    wo_copy(0).start()
    for j in range(2, 6):
        wmod_copy(j).start()
    for g in range(1, _HKV):
        wo_copy(g).start()
    for t in range(1, _NT):
        x_copy(t).start()

    k_copy.wait()
    for g in range(_HKV):
        kt_vmem[g] = k_vmem[g].astype(_F32).T.astype(_BF)
    v_copy.wait()

    best_smem[0] = jnp.float32(-jnp.inf)
    bidx_smem[0] = jnp.int32(0)

    wr = wr_ref[...].astype(_F32)
    row_iota = jax.lax.broadcasted_iota(jnp.int32, (_TM, 1), 0)

    def tile_body(t, carry):
        r0 = pl.multiple_of(t * _TM, _TM)
        rows = pl.ds(r0, _TM)
        first = t == 0

        @pl.when(t == 1)
        def _():
            wg_copy.start()
            wu_copy.start()
            wd_copy.start()

        x_copy(t).wait()
        sa = mod_scr[0:1, :] * _QSCALE
        ca = (1.0 + mod_scr[1:2, :]) * _QSCALE
        x = x_vmem[rows, :].astype(_F32)
        h_scr[...] = (_layernorm(x) * ca + sa).astype(_BF)

        for g in range(_HKV):
            @pl.when(first)
            def _():
                wq_copy(g).wait()
            q = jnp.dot(h_scr[...], wq_vmem[:, g * _GW:(g + 1) * _GW],
                        preferred_element_type=_F32).astype(_BF)
            for j in range(_REP):
                s = jnp.dot(q[:, j * _DH:(j + 1) * _DH], kt_vmem[g],
                            preferred_element_type=_F32)
                m = jnp.max(s, axis=-1, keepdims=True)
                p = jnp.exp2(s - m)
                l = jnp.sum(p, axis=-1, keepdims=True)
                o = jnp.dot(p.astype(_BF), v_vmem[g],
                            preferred_element_type=_F32)
                o_scr[:, j * _DH:(j + 1) * _DH] = (o * (1.0 / l)).astype(_BF)

            @pl.when(first)
            def _():
                wo_copy(g).wait()
            a = jnp.dot(o_scr[...], wo_vmem[g * _GW:(g + 1) * _GW, :],
                        preferred_element_type=_F32)
            if g == 0:
                acc_scr[...] = a
            else:
                acc_scr[...] += a

        @pl.when(first)
        def _():
            for j in range(2, 6):
                mod_chunk(j)

        ga = mod_scr[2:3, :]
        sb = mod_scr[3:4, :]
        cb = 1.0 + mod_scr[4:5, :]
        gb = mod_scr[5:6, :]
        x1 = x_vmem[rows, :].astype(_F32) + ga * acc_scr[...]
        h2 = (_layernorm(x1) * cb + sb).astype(_BF)
        h2_vmem[rows, :] = h2
        h2f = h2.astype(_F32)
        out_vmem[rows, :] = (x1 + gb * h2f).astype(_BF)
        out_copy(t).start()

        r = jnp.sum(h2f * wr, axis=-1, keepdims=True).astype(_BF).astype(_F32)
        rmax = jnp.max(r)
        ridx = jnp.min(jnp.where(r == rmax, row_iota, _TM))

        @pl.when(rmax > best_smem[0])
        def _():
            best_smem[0] = rmax
            bidx_smem[0] = r0 + ridx

        return carry

    jax.lax.fori_loop(0, _NT, tile_body, 0)

    idx = bidx_smem[0]
    base = pl.multiple_of((idx // 16) * 16, 16)
    sel = jax.lax.broadcasted_iota(jnp.int32, (16, 1), 0) == (idx - base)
    h2blk = h2_vmem[pl.ds(base, 16), :]
    wg_copy.wait()
    wu_copy.wait()
    g = jnp.dot(h2blk, wg_vmem[...], preferred_element_type=_F32)
    u = jnp.dot(h2blk, wu_vmem[...], preferred_element_type=_F32)
    gu = (_silu(g) * u).astype(_BF)
    wd_copy.wait()
    y = jnp.dot(gu, wd_vmem[...], preferred_element_type=_F32)
    y = y * jax.nn.sigmoid(jnp.full((1, _D), best_smem[0], _F32))
    gb = mod_scr[5:6, :]
    for t in range(_NT):
        out_copy(t).wait()
    blk = out_vmem[pl.ds(base, 16), :].astype(_F32)
    blk = jnp.where(sel, blk + gb * y, blk)
    out_vmem[pl.ds(base, 16), :] = blk.astype(_BF)
    fix = pltpu.make_async_copy(
        out_vmem.at[pl.ds(base, 16), :],
        out_hbm.at[0, pl.ds(base, 16), :],
        fix_sem)
    fix.start()
    fix.wait()


@jax.jit
def pallas_adaLN_cond__sliding_block_cached__moe_arch_mod__prompt_kernel(
    A_x: jax.Array,
    A_k_cache: jax.Array,
    A_v_cache: jax.Array,
    A_wq: jax.Array,
    A_wo: jax.Array,
    B_x: jax.Array,
    B_w_r: jax.Array,
    B_w_gate: jax.Array,
    B_w_up: jax.Array,
    B_w_down: jax.Array,
    c: jax.Array,
    w_mod: jax.Array,
):
    del B_x
    any_spec = pl.BlockSpec(memory_space=pl.ANY)
    vmem_spec = pl.BlockSpec(memory_space=pltpu.VMEM)
    return pl.pallas_call(
        _kernel,
        out_shape=jax.ShapeDtypeStruct(A_x.shape, A_x.dtype),
        in_specs=[
            any_spec, any_spec, any_spec, any_spec, any_spec,
            vmem_spec,
            any_spec, any_spec, any_spec,
            vmem_spec,
            any_spec,
        ],
        out_specs=any_spec,
        scratch_shapes=[
            pltpu.VMEM((_S, _D), _BF),
            pltpu.VMEM((_S, _D), _BF),
            pltpu.VMEM((_S, _D), _BF),
            pltpu.VMEM((_HKV, _W, _DH), _BF),
            pltpu.VMEM((_HKV, _DH, _W), _BF),
            pltpu.VMEM((_HKV, _W, _DH), _BF),
            pltpu.VMEM((_D, _HQ * _DH), _BF),
            pltpu.VMEM((_HQ * _DH, _D), _BF),
            pltpu.VMEM((_D, 6 * _D), _BF),
            pltpu.VMEM((_D, _F), _BF),
            pltpu.VMEM((_D, _F), _BF),
            pltpu.VMEM((_F, _D), _BF),
            pltpu.VMEM((_TM, _D), _BF),
            pltpu.VMEM((_TM, _GW), _BF),
            pltpu.VMEM((_TM, _D), _F32),
            pltpu.VMEM((8, _D), _F32),
            pltpu.SMEM((1,), _F32),
            pltpu.SMEM((1,), jnp.int32),
            pltpu.SemaphoreType.DMA((_NT,)),
            pltpu.SemaphoreType.DMA((_NT,)),
            pltpu.SemaphoreType.DMA((2,)),
            pltpu.SemaphoreType.DMA((_HKV,)),
            pltpu.SemaphoreType.DMA((_HKV,)),
            pltpu.SemaphoreType.DMA((6,)),
            pltpu.SemaphoreType.DMA((3,)),
            pltpu.SemaphoreType.DMA(()),
        ],
        compiler_params=pltpu.CompilerParams(
            vmem_limit_bytes=110 * 1024 * 1024,
        ),
    )(A_x, A_k_cache, A_v_cache, A_wq, A_wo, B_w_r.reshape(1, _D),
      B_w_gate, B_w_up, B_w_down, c, w_mod)
```

```python
import math

import jax
import jax.numpy as jnp
import jax.experimental.pallas as pl
import jax.experimental.pallas.tpu as pltpu

_S = 2048
_D = 1024
_HQ = 32
_HKV = 4
_DH = 128
_SK = 2048
_W = 512
_F = 3584
_REP = _HQ // _HKV
_GW = _REP * _DH
_TM = 512
_NT = _S // _TM
_HP = 2
_NSTEP = _REP // _HP
_CH = 64
_LINK = False
_EPS = 1e-5
_QSCALE = (_DH ** -0.5) * math.log2(math.e)

_BF = jnp.bfloat16
_F32 = jnp.float32


def _layernorm(x):
    inv_n = 1.0 / x.shape[-1]
    m = jnp.sum(x, axis=-1, keepdims=True) * inv_n
    xc = x - m
    v = jnp.sum(xc * xc, axis=-1, keepdims=True) * inv_n
    return xc * jax.lax.rsqrt(v + _EPS)


def _recip(x):
    r = pl.reciprocal(x, approx=True)
    return r * (2.0 - x * r)


def _silu(x):
    return x * jax.nn.sigmoid(x)


def _kernel(
    x_hbm, k_hbm, v_hbm, wq_hbm, wo_hbm, wr_ref, wg_hbm, wu_hbm, wd_hbm, c_ref,
    wmod_hbm,
    out_hbm,
    x_vmem, out_vmem, h2_vmem, k_vmem, kt_vmem, v_vmem, wq_vmem, wo_vmem,
    wmod_vmem, wg_vmem, wu_vmem, wd_vmem, h_scr,
    x_sem, out_sem, kv_sem, wq_sem, wqp_sem, wo_sem, wmod_sem, ffn_sem, fix_sem,
):
    def x_copy(t):
        return pltpu.make_async_copy(
            x_hbm.at[0, pl.ds(t * _TM, _TM), :],
            x_vmem.at[pl.ds(t * _TM, _TM), :],
            x_sem.at[t])

    def out_copy(t):
        return pltpu.make_async_copy(
            out_vmem.at[pl.ds(t * _TM, _TM), :],
            out_hbm.at[0, pl.ds(t * _TM, _TM), :],
            out_sem.at[t])

    def wmod_copy(j):
        return pltpu.make_async_copy(
            wmod_hbm.at[:, pl.ds(j * _D, _D)],
            wmod_vmem.at[:, pl.ds(j * _D, _D)],
            wmod_sem.at[j])

    def wq_copy(g):
        return pltpu.make_async_copy(
            wq_hbm.at[:, pl.ds(g * _GW, _GW)],
            wq_vmem.at[:, pl.ds(g * _GW, _GW)],
            wq_sem.at[g])

    def wqp_copy(i):
        n = _HP * _DH
        return pltpu.make_async_copy(
            wq_hbm.at[:, pl.ds(i * n, n)],
            wq_vmem.at[:, pl.ds(i * n, n)],
            wqp_sem.at[i])

    def wo_copy(g):
        return pltpu.make_async_copy(
            wo_hbm.at[pl.ds(g * _GW, _GW), :],
            wo_vmem.at[pl.ds(g * _GW, _GW), :],
            wo_sem.at[g])

    k_copy = pltpu.make_async_copy(
        k_hbm.at[0, :, pl.ds(_SK - _W, _W), :], k_vmem, kv_sem.at[0])
    v_copy = pltpu.make_async_copy(
        v_hbm.at[0, :, pl.ds(_SK - _W, _W), :], v_vmem, kv_sem.at[1])
    wg_copy = pltpu.make_async_copy(wg_hbm, wg_vmem, ffn_sem.at[0])
    wu_copy = pltpu.make_async_copy(wu_hbm, wu_vmem, ffn_sem.at[1])
    wd_copy = pltpu.make_async_copy(wd_hbm, wd_vmem, ffn_sem.at[2])

    c = c_ref[...].astype(_F32)
    sc = jnp.broadcast_to(_silu(c), (16, _D)).astype(_BF)
    wr = wr_ref[...].astype(_F32).reshape(1, _D)
    sub_iota = jax.lax.broadcasted_iota(jnp.int32, (8, 1), 0)
    neg_inf = pl.semaphore_read(fix_sem).astype(_F32) - jnp.inf

    def link(*vals):
        acc = None
        for v in vals:
            u = pltpu.bitcast(v, jnp.int32)
            for r in range(u.shape[0] // 8):
                for cc in range(u.shape[1] // 128):
                    blk = u[r * 8:(r + 1) * 8, cc * 128:(cc + 1) * 128]
                    acc = blk if acc is None else jnp.maximum(acc, blk)
        return pltpu.bitcast(acc, _F32) < neg_inf

    def mod_chunk(j):
        r = jnp.dot(sc, wmod_vmem[:, j * _D:(j + 1) * _D],
                    preferred_element_type=_F32)
        return r[0:1, :]

    def ln1(t, sa, ca, mask):
        n = _CH
        for r0 in range(0, _TM, n):
            x = x_vmem[t * _TM + r0:t * _TM + r0 + n, :].astype(_F32)
            if mask is not None:
                x = jnp.where(jnp.tile(mask, (n // 8, _D // 128)), 0.0, x)
            hb = (_layernorm(x) * ca + sa).astype(_BF)
            h_scr[t % 2, r0:r0 + n, :] = hb
            mask = link(hb) if _LINK else None
        return mask

    def qpiece(h, g, i):
        c0 = g * _GW + i * _HP * _DH
        return jnp.dot(h_scr[h], wq_vmem[:, c0:c0 + _HP * _DH],
                       preferred_element_type=_F32).astype(_BF)

    def opiece(o, g, i):
        c0 = i * _HP * _DH
        return jnp.dot(o, wo_vmem[g * _GW:(g + 1) * _GW, c0:c0 + _HP * _DH],
                       preferred_element_type=_F32)

    state = {"best_v": jnp.full((8, 1), -jnp.inf, _F32),
             "best_i": jnp.zeros((8, 1), jnp.int32)}

    def epilogue(t, acc, mods, mask):
        ga, sb, cb, gb = mods
        n = _CH
        ga8 = jnp.broadcast_to(ga, (8, _D))
        for c0 in range(0, _TM, n):
            r0 = t * _TM + c0
            gam = ga8
            if mask is not None:
                gam = jnp.where(jnp.tile(mask, (1, _D // 128)), 0.0, ga8)
            x1 = (x_vmem[r0:r0 + n, :].astype(_F32)
                  + jnp.tile(gam, (n // 8, 1)) * acc[c0:c0 + n, :])
            h2 = _layernorm(x1) * cb + sb
            h2b = h2.astype(_BF)
            outb = (x1 + gb * h2).astype(_BF)
            h2_vmem[r0:r0 + n, :] = h2b
            out_vmem[r0:r0 + n, :] = outb
            mask = link(h2b, outb) if _LINK else None
            r = jnp.sum(h2 * wr, axis=-1, keepdims=True)
            bv, bi = state["best_v"], state["best_i"]
            for k in range(n // 8):
                rk = r[k * 8:(k + 1) * 8, :]
                gt = rk > bv
                bv = jnp.where(gt, rk, bv)
                bi = jnp.where(gt, sub_iota + (r0 + k * 8), bi)
            state["best_v"], state["best_i"] = bv, bi
        return mask

    def step_attn(q, g, i, h, gq, o_prev, g_prev, acc, side):
        ss = []
        for j in range(i * _HP, (i + 1) * _HP):
            ss.append(jnp.dot(q[:, j * _DH:(j + 1) * _DH], kt_vmem[g],
                              preferred_element_type=_F32))
        qn = qpiece(h, gq, i) if h is not None else None
        for f in side:
            f()
        outs = []
        for s in ss:
            m = jnp.max(s, axis=-1, keepdims=True)
            p = jnp.exp2(s - m)
            l = jnp.sum(p, axis=-1, keepdims=True)
            o = jnp.dot(p.astype(_BF), v_vmem[g],
                        preferred_element_type=_F32)
            outs.append((o * _recip(l)).astype(_BF))
        a = None
        if o_prev is not None:
            a = opiece(o_prev, g_prev, i)
            if acc is not None:
                a = acc + a
        return qn, outs, a

    x_copy(0).start()
    wmod_copy(1).start()
    x_copy(0).wait()
    wmod_copy(0).start()
    xhat = _layernorm(x_vmem[0:_TM, :].astype(_F32))
    wmod_copy(1).wait()
    wqp_copy(0).start()
    ca = (1.0 + mod_chunk(1)) * _QSCALE
    wmod_copy(0).wait()
    for i in range(1, _NSTEP):
        wqp_copy(i).start()
    sa = mod_chunk(0) * _QSCALE
    h_scr[0] = (xhat * ca + sa).astype(_BF)
    h = 0
    qs = []
    for i in range(_NSTEP):
        wqp_copy(i).wait()
        if i == 0:
            k_copy.start()
            v_copy.start()
        if i == 1:
            wq_copy(1).start()
        if i == 3:
            wo_copy(0).start()
            x_copy(1).start()
            wq_copy(2).start()
        qs.append(qpiece(h, 0, i))
    q = jnp.concatenate(qs, axis=1)
    k_copy.wait()
    for g in range(_HKV):
        kt_vmem[g] = k_vmem[g].astype(_F32).T.astype(_BF)
    v_copy.wait()

    ngrp = _NT * _HKV
    mods = [None] * 6
    acc = [None] * _NSTEP
    o_prev = None
    mask = None
    for n in range(ngrp):
        t, g = divmod(n, _HKV)
        tn, gn = divmod(n + 1, _HKV)
        gp = (n - 1) % _HKV
        if n == 0:
            wq_copy(1).wait()
        elif n == 1:
            wo_copy(0).wait()
            wq_copy(2).wait()
            wo_copy(1).start()
            wq_copy(3).start()
            wo_copy(2).start()
        elif n == 2:
            wo_copy(1).wait()
            wq_copy(3).wait()
            wo_copy(3).start()
            for j in range(2, 6):
                wmod_copy(j).start()
        elif n == 3:
            wo_copy(2).wait()
            for tt in range(2, _NT):
                x_copy(tt).start()
        elif n == 4:
            wo_copy(3).wait()
            for j in range(2, 6):
                wmod_copy(j).wait()
            wg_copy.start()
            wu_copy.start()
            wd_copy.start()
        if g == 1:
            mask = None
            if t + 1 < _NT:
                x_copy(t + 1).wait()
            if t >= 1:
                mask = epilogue(t - 1, jnp.concatenate(acc_fin, axis=1),
                                mods[2:], None)
            if t + 1 < _NT:
                mask = ln1(t + 1, sa, ca, mask)
        if g == 3 and t >= 1:
            out_copy(t - 1).start()

        if gn == 0 and tn < _NT:
            h = tn % 2
        if gp == 0:
            acc = [None] * _NSTEP
        q_next, outs = [], []
        for i in range(_NSTEP):
            side = []
            if n == 4:
                def _mod(i=i):
                    r = mod_chunk(2 + i)
                    mods[2 + i] = 1.0 + r if i == 2 else r
                side.append(_mod)
            qn, o_i, a = step_attn(q, g, i, h if tn < _NT else None, gn,
                                   o_prev, gp, acc[i], side)
            q_next.append(qn)
            outs.extend(o_i)
            acc[i] = a
        if gp == _HKV - 1 and n >= 1:
            acc_fin = acc
        o_prev = jnp.concatenate(outs, axis=1)
        if tn < _NT:
            q = jnp.concatenate(q_next, axis=1)
    acc = [acc[i] + opiece(o_prev, _HKV - 1, i) for i in range(_NSTEP)]
    epilogue(_NT - 1, jnp.concatenate(acc, axis=1), mods[2:], mask)
    out_copy(_NT - 1).start()
    gb = mods[5]
    bv, bi = state["best_v"], state["best_i"]
    best_r = jnp.max(bv)
    idx = jnp.min(jnp.where(bv == best_r, bi, _S))

    base = pl.multiple_of((idx // 16) * 16, 16)
    sel = jax.lax.broadcasted_iota(jnp.int32, (16, 1), 0) == (idx - base)
    h2blk = h2_vmem[pl.ds(base, 16), :]
    wg_copy.wait()
    wu_copy.wait()
    g = jnp.dot(h2blk, wg_vmem[...], preferred_element_type=_F32)
    u = jnp.dot(h2blk, wu_vmem[...], preferred_element_type=_F32)
    gu = (_silu(g) * u).astype(_BF)
    wd_copy.wait()
    y = jnp.dot(gu, wd_vmem[...], preferred_element_type=_F32)
    y = y * jax.nn.sigmoid(jnp.full((1, _D), best_r, _F32))
    for t in range(_NT):
        out_copy(t).wait()
    blk = out_vmem[pl.ds(base, 16), :].astype(_F32)
    blk = jnp.where(sel, blk + gb * y, blk)
    out_vmem[pl.ds(base, 16), :] = blk.astype(_BF)
    fix = pltpu.make_async_copy(
        out_vmem.at[pl.ds(base, 16), :],
        out_hbm.at[0, pl.ds(base, 16), :],
        fix_sem)
    fix.start()
    fix.wait()


@jax.jit
def pallas_adaLN_cond__sliding_block_cached__moe_arch_mod__prompt_kernel(
    A_x: jax.Array,
    A_k_cache: jax.Array,
    A_v_cache: jax.Array,
    A_wq: jax.Array,
    A_wo: jax.Array,
    B_x: jax.Array,
    B_w_r: jax.Array,
    B_w_gate: jax.Array,
    B_w_up: jax.Array,
    B_w_down: jax.Array,
    c: jax.Array,
    w_mod: jax.Array,
):
    del B_x
    any_spec = pl.BlockSpec(memory_space=pl.ANY)
    vmem_spec = pl.BlockSpec(memory_space=pltpu.VMEM)
    return pl.pallas_call(
        _kernel,
        out_shape=jax.ShapeDtypeStruct(A_x.shape, A_x.dtype),
        in_specs=[
            any_spec, any_spec, any_spec, any_spec, any_spec,
            vmem_spec,
            any_spec, any_spec, any_spec,
            vmem_spec,
            any_spec,
        ],
        out_specs=any_spec,
        scratch_shapes=[
            pltpu.VMEM((_S, _D), _BF),
            pltpu.VMEM((_S, _D), _BF),
            pltpu.VMEM((_S, _D), _BF),
            pltpu.VMEM((_HKV, _W, _DH), _BF),
            pltpu.VMEM((_HKV, _DH, _W), _BF),
            pltpu.VMEM((_HKV, _W, _DH), _BF),
            pltpu.VMEM((_D, _HQ * _DH), _BF),
            pltpu.VMEM((_HQ * _DH, _D), _BF),
            pltpu.VMEM((_D, 6 * _D), _BF),
            pltpu.VMEM((_D, _F), _BF),
            pltpu.VMEM((_D, _F), _BF),
            pltpu.VMEM((_F, _D), _BF),
            pltpu.VMEM((2, _TM, _D), _BF),
            pltpu.SemaphoreType.DMA((_NT,)),
            pltpu.SemaphoreType.DMA((_NT,)),
            pltpu.SemaphoreType.DMA((2,)),
            pltpu.SemaphoreType.DMA((_HKV,)),
            pltpu.SemaphoreType.DMA((_NSTEP,)),
            pltpu.SemaphoreType.DMA((_HKV,)),
            pltpu.SemaphoreType.DMA((6,)),
            pltpu.SemaphoreType.DMA((3,)),
            pltpu.SemaphoreType.DMA(()),
        ],
        compiler_params=pltpu.CompilerParams(
            vmem_limit_bytes=110 * 1024 * 1024,
        ),
    )(A_x, A_k_cache, A_v_cache, A_wq, A_wo, B_w_r,
      B_w_gate, B_w_up, B_w_down, c, w_mod)
```

```python
import math

import jax
import jax.numpy as jnp
import jax.experimental.pallas as pl
import jax.experimental.pallas.tpu as pltpu

_S = 2048
_D = 1024
_HQ = 32
_HKV = 4
_DH = 128
_SK = 2048
_W = 512
_F = 3584
_REP = _HQ // _HKV
_GW = _REP * _DH
_TM = 512
_NT = _S // _TM
_HP = 2
_NSTEP = _REP // _HP
_CH = 64
_LINK = False
_NMK = 4
_MK = _D // _NMK
_FB = 4
_EPS = 1e-5
_QSCALE = (_DH ** -0.5) * math.log2(math.e)

_BF = jnp.bfloat16
_F32 = jnp.float32


def _layernorm(x):
    inv_n = 1.0 / x.shape[-1]
    m = jnp.sum(x, axis=-1, keepdims=True) * inv_n
    xc = x - m
    v = jnp.sum(xc * xc, axis=-1, keepdims=True) * inv_n
    return xc * jax.lax.rsqrt(v + _EPS)


def _recip(x):
    return pl.reciprocal(x, approx=True)


def _silu(x):
    return x * jax.nn.sigmoid(x)


def _kernel(
    x_hbm, k_hbm, v_hbm, wq_hbm, wo_hbm, wr_ref, wg_hbm, wu_hbm, wd_hbm, c_ref,
    wmod_hbm,
    out_hbm,
    x_vmem, out_vmem, h2_vmem, k_vmem, kt_vmem, v_vmem, wq_vmem, wo_vmem,
    wmod_vmem, wg_vmem, wu_vmem, wd_vmem, h_scr,
    x_sem, out_sem, kv_sem, wq_sem, wqp_sem, wo_sem, wmod_sem, ffn_sem, fix_sem,
):
    def x_copy(t):
        return pltpu.make_async_copy(
            x_hbm.at[0, pl.ds(t * _TM, _TM), :],
            x_vmem.at[pl.ds(t * _TM, _TM), :],
            x_sem.at[t])

    def out_copy(t):
        return pltpu.make_async_copy(
            out_vmem.at[pl.ds(t * _TM, _TM), :],
            out_hbm.at[0, pl.ds(t * _TM, _TM), :],
            out_sem.at[t])

    def wmodA_copy(i):
        rows = pl.ds(i * _MK, _MK)
        return pltpu.make_async_copy(
            wmod_hbm.at[rows, pl.ds(0, 2 * _D)],
            wmod_vmem.at[rows, pl.ds(0, 2 * _D)],
            wmod_sem.at[i])

    def wmodB_copy(i):
        cols = pl.ds(2 * _D + i * 2 * _D, 2 * _D)
        return pltpu.make_async_copy(
            wmod_hbm.at[:, cols], wmod_vmem.at[:, cols],
            wmod_sem.at[_NMK + i])

    def wq_copy(g):
        return pltpu.make_async_copy(
            wq_hbm.at[:, pl.ds(g * _GW, _GW)],
            wq_vmem.at[:, pl.ds(g * _GW, _GW)],
            wq_sem.at[g])

    def wqp_copy(i):
        n = _HP * _DH
        return pltpu.make_async_copy(
            wq_hbm.at[:, pl.ds(i * n, n)],
            wq_vmem.at[:, pl.ds(i * n, n)],
            wqp_sem.at[i])

    def wo_copy(g):
        return pltpu.make_async_copy(
            wo_hbm.at[pl.ds(g * _GW, _GW), :],
            wo_vmem.at[pl.ds(g * _GW, _GW), :],
            wo_sem.at[g])

    k_copy = pltpu.make_async_copy(
        k_hbm.at[0, :, pl.ds(_SK - _W, _W), :], k_vmem, kv_sem.at[0])
    v_copy = pltpu.make_async_copy(
        v_hbm.at[0, :, pl.ds(_SK - _W, _W), :], v_vmem, kv_sem.at[1])
    wg_copy = pltpu.make_async_copy(wg_hbm, wg_vmem, ffn_sem.at[0])
    wu_copy = pltpu.make_async_copy(wu_hbm, wu_vmem, ffn_sem.at[1])
    wd_copy = pltpu.make_async_copy(wd_hbm, wd_vmem, ffn_sem.at[2])

    c = c_ref[...].astype(_F32)
    sc = jnp.broadcast_to(_silu(c), (16, _D)).astype(_BF)
    wr = wr_ref[...].astype(_F32).reshape(1, _D)
    sub_iota = jax.lax.broadcasted_iota(jnp.int32, (8, 1), 0)
    neg_inf = pl.semaphore_read(fix_sem).astype(_F32) - jnp.inf

    def link(*vals):
        acc = None
        for v in vals:
            u = pltpu.bitcast(v, jnp.int32)
            for r in range(u.shape[0] // 8):
                for cc in range(u.shape[1] // 128):
                    blk = u[r * 8:(r + 1) * 8, cc * 128:(cc + 1) * 128]
                    acc = blk if acc is None else jnp.maximum(acc, blk)
        return pltpu.bitcast(acc, _F32) < neg_inf

    def mod_chunk(j):
        r = jnp.dot(sc, wmod_vmem[:, j * _D:(j + 1) * _D],
                    preferred_element_type=_F32)
        return r[0:1, :]

    def ln1(t, sa, ca, mask):
        n = _CH
        for r0 in range(0, _TM, n):
            x = x_vmem[t * _TM + r0:t * _TM + r0 + n, :].astype(_F32)
            if mask is not None:
                x = jnp.where(jnp.tile(mask, (n // 8, _D // 128)), 0.0, x)
            hb = (_layernorm(x) * ca + sa).astype(_BF)
            h_scr[t % 2, r0:r0 + n, :] = hb
            mask = link(hb) if _LINK else None
        return mask

    def qpiece(h, g, i):
        c0 = g * _GW + i * _HP * _DH
        return jnp.dot(h_scr[h], wq_vmem[:, c0:c0 + _HP * _DH],
                       preferred_element_type=_F32).astype(_BF)

    def opiece(o, g, i):
        c0 = i * _HP * _DH
        return jnp.dot(o, wo_vmem[g * _GW:(g + 1) * _GW, c0:c0 + _HP * _DH],
                       preferred_element_type=_F32)

    state = {"best_v": jnp.full((8, 1), -jnp.inf, _F32),
             "best_i": jnp.zeros((8, 1), jnp.int32)}

    def epilogue(t, acc, mods, mask):
        ga, sb, cb, gb = mods
        n = _CH
        ga8 = jnp.broadcast_to(ga, (8, _D))
        for c0 in range(0, _TM, n):
            r0 = t * _TM + c0
            gam = ga8
            if mask is not None:
                gam = jnp.where(jnp.tile(mask, (1, _D // 128)), 0.0, ga8)
            x1 = (x_vmem[r0:r0 + n, :].astype(_F32)
                  + jnp.tile(gam, (n // 8, 1)) * acc[c0:c0 + n, :])
            h2 = _layernorm(x1) * cb + sb
            h2b = h2.astype(_BF)
            outb = (x1 + gb * h2).astype(_BF)
            h2_vmem[r0:r0 + n, :] = h2b
            out_vmem[r0:r0 + n, :] = outb
            mask = link(h2b, outb) if _LINK else None
            r = jnp.sum(h2 * wr, axis=-1, keepdims=True)
            bv, bi = state["best_v"], state["best_i"]
            for k in range(n // 8):
                rk = r[k * 8:(k + 1) * 8, :]
                gt = rk > bv
                bv = jnp.where(gt, rk, bv)
                bi = jnp.where(gt, sub_iota + (r0 + k * 8), bi)
            state["best_v"], state["best_i"] = bv, bi
        return mask

    def step_attn(q, g, i, h, gq, o_prev, g_prev, acc, side):
        ss = []
        for j in range(i * _HP, (i + 1) * _HP):
            ss.append(jnp.dot(q[:, j * _DH:(j + 1) * _DH], kt_vmem[g],
                              preferred_element_type=_F32))
        qn = qpiece(h, gq, i) if h is not None else None
        for f in side:
            f()
        outs = []
        for s in ss:
            m = jnp.max(s, axis=-1, keepdims=True)
            p = jnp.exp2(s - m)
            l = jnp.sum(p, axis=-1, keepdims=True)
            o = jnp.dot(p.astype(_BF), v_vmem[g],
                        preferred_element_type=_F32)
            outs.append((o * _recip(l)).astype(_BF))
        a = None
        if o_prev is not None:
            a = opiece(o_prev, g_prev, i)
            if acc is not None:
                a = acc + a
        return qn, outs, a

    x_copy(0).start()
    wmodA_copy(0).start()
    x_copy(0).wait()
    wmodA_copy(1).start()
    wmodA_copy(2).start()
    xhat = _layernorm(x_vmem[0:_TM, :].astype(_F32))
    modA = None
    for i in range(_NMK):
        wmodA_copy(i).wait()
        if i == 0:
            wmodA_copy(3).start()
        elif i == 2:
            wqp_copy(0).start()
        elif i == 3:
            wqp_copy(1).start()
            wqp_copy(2).start()
        part = jnp.dot(sc[:, i * _MK:(i + 1) * _MK],
                       wmod_vmem[i * _MK:(i + 1) * _MK, 0:2 * _D],
                       preferred_element_type=_F32)
        modA = part if modA is None else modA + part
    sa = modA[0:1, 0:_D] * _QSCALE
    ca = (1.0 + modA[0:1, _D:2 * _D]) * _QSCALE
    h_scr[0] = (xhat * ca + sa).astype(_BF)
    h = 0
    qs = []
    for i in range(_NSTEP):
        wqp_copy(i).wait()
        if i == 0:
            wqp_copy(3).start()
            k_copy.start()
            v_copy.start()
        if i == 1:
            wq_copy(1).start()
        if i == 3:
            wo_copy(0).start()
            x_copy(1).start()
            wq_copy(2).start()
        qs.append(qpiece(h, 0, i))
    q = jnp.concatenate(qs, axis=1)
    k_copy.wait()
    for g in range(_HKV):
        kt_vmem[g] = k_vmem[g].astype(_F32).T.astype(_BF)
    v_copy.wait()

    ngrp = _NT * _HKV
    mods = [None] * 6
    acc = [None] * _NSTEP
    o_prev = None
    mask = None
    for n in range(ngrp):
        t, g = divmod(n, _HKV)
        tn, gn = divmod(n + 1, _HKV)
        gp = (n - 1) % _HKV
        if n == 0:
            wq_copy(1).wait()
        elif n == 1:
            wo_copy(0).wait()
            wq_copy(2).wait()
            wo_copy(1).start()
            wq_copy(3).start()
            wo_copy(2).start()
        elif n == 2:
            wo_copy(1).wait()
            wq_copy(3).wait()
            wo_copy(3).start()
            wmodB_copy(0).start()
            wmodB_copy(1).start()
        elif n == 3:
            wo_copy(2).wait()
            for tt in range(2, _NT):
                x_copy(tt).start()
        elif n == 4:
            wo_copy(3).wait()
            wmodB_copy(0).wait()
            wmodB_copy(1).wait()
            wg_copy.start()
            wu_copy.start()
            wd_copy.start()
        if g == 1:
            mask = None
            if t + 1 < _NT:
                x_copy(t + 1).wait()
            if t >= 1:
                mask = epilogue(t - 1, jnp.concatenate(acc_fin, axis=1),
                                mods[2:], None)
            if t + 1 < _NT:
                mask = ln1(t + 1, sa, ca, mask)
        if g == 3 and t >= 1:
            out_copy(t - 1).start()

        if gn == 0 and tn < _NT:
            h = tn % 2
        if gp == 0:
            acc = [None] * _NSTEP
        q_next, outs = [], []
        for i in range(_NSTEP):
            side = []
            if n == 4:
                def _mod(i=i):
                    r = mod_chunk(2 + i)
                    mods[2 + i] = 1.0 + r if i == 2 else r
                side.append(_mod)
            qn, o_i, a = step_attn(q, g, i, h if tn < _NT else None, gn,
                                   o_prev, gp, acc[i], side)
            q_next.append(qn)
            outs.extend(o_i)
            acc[i] = a
        if gp == _HKV - 1 and n >= 1:
            acc_fin = acc
        o_prev = jnp.concatenate(outs, axis=1)
        if tn < _NT:
            q = jnp.concatenate(q_next, axis=1)
    acc = [acc[i] + opiece(o_prev, _HKV - 1, i) for i in range(_NSTEP)]
    epilogue(_NT - 1, jnp.concatenate(acc, axis=1), mods[2:], mask)
    out_copy(_NT - 1).start()
    gb = mods[5]
    bv, bi = state["best_v"], state["best_i"]
    best_r = jnp.max(bv)
    idx = jnp.min(jnp.where(bv == best_r, bi, _S))

    base = pl.multiple_of((idx // 16) * 16, 16)
    sel = jax.lax.broadcasted_iota(jnp.int32, (16, 1), 0) == (idx - base)
    h2blk = h2_vmem[pl.ds(base, 16), :]
    wg_copy.wait()
    wu_copy.wait()
    wd_copy.wait()
    y = None
    fb = _F // _FB
    for i in range(_FB):
        fs = slice(i * fb, (i + 1) * fb)
        g = jnp.dot(h2blk, wg_vmem[:, fs], preferred_element_type=_F32)
        u = jnp.dot(h2blk, wu_vmem[:, fs], preferred_element_type=_F32)
        gu = (_silu(g) * u).astype(_BF)
        part = jnp.dot(gu, wd_vmem[fs, :], preferred_element_type=_F32)
        y = part if y is None else y + part
    y = y * jax.nn.sigmoid(jnp.full((1, _D), best_r, _F32))
    for t in range(_NT):
        out_copy(t).wait()
    blk = out_vmem[pl.ds(base, 16), :].astype(_F32)
    blk = jnp.where(sel, blk + gb * y, blk)
    out_vmem[pl.ds(base, 16), :] = blk.astype(_BF)
    fix = pltpu.make_async_copy(
        out_vmem.at[pl.ds(base, 16), :],
        out_hbm.at[0, pl.ds(base, 16), :],
        fix_sem)
    fix.start()
    fix.wait()


@jax.jit
def pallas_adaLN_cond__sliding_block_cached__moe_arch_mod__prompt_kernel(
    A_x: jax.Array,
    A_k_cache: jax.Array,
    A_v_cache: jax.Array,
    A_wq: jax.Array,
    A_wo: jax.Array,
    B_x: jax.Array,
    B_w_r: jax.Array,
    B_w_gate: jax.Array,
    B_w_up: jax.Array,
    B_w_down: jax.Array,
    c: jax.Array,
    w_mod: jax.Array,
):
    del B_x
    any_spec = pl.BlockSpec(memory_space=pl.ANY)
    vmem_spec = pl.BlockSpec(memory_space=pltpu.VMEM)
    return pl.pallas_call(
        _kernel,
        out_shape=jax.ShapeDtypeStruct(A_x.shape, A_x.dtype),
        in_specs=[
            any_spec, any_spec, any_spec, any_spec, any_spec,
            vmem_spec,
            any_spec, any_spec, any_spec,
            vmem_spec,
            any_spec,
        ],
        out_specs=any_spec,
        scratch_shapes=[
            pltpu.VMEM((_S, _D), _BF),
            pltpu.VMEM((_S, _D), _BF),
            pltpu.VMEM((_S, _D), _BF),
            pltpu.VMEM((_HKV, _W, _DH), _BF),
            pltpu.VMEM((_HKV, _DH, _W), _BF),
            pltpu.VMEM((_HKV, _W, _DH), _BF),
            pltpu.VMEM((_D, _HQ * _DH), _BF),
            pltpu.VMEM((_HQ * _DH, _D), _BF),
            pltpu.VMEM((_D, 6 * _D), _BF),
            pltpu.VMEM((_D, _F), _BF),
            pltpu.VMEM((_D, _F), _BF),
            pltpu.VMEM((_F, _D), _BF),
            pltpu.VMEM((2, _TM, _D), _BF),
            pltpu.SemaphoreType.DMA((_NT,)),
            pltpu.SemaphoreType.DMA((_NT,)),
            pltpu.SemaphoreType.DMA((2,)),
            pltpu.SemaphoreType.DMA((_HKV,)),
            pltpu.SemaphoreType.DMA((_NSTEP,)),
            pltpu.SemaphoreType.DMA((_HKV,)),
            pltpu.SemaphoreType.DMA((_NMK + 2,)),
            pltpu.SemaphoreType.DMA((3,)),
            pltpu.SemaphoreType.DMA(()),
        ],
        compiler_params=pltpu.CompilerParams(
            vmem_limit_bytes=110 * 1024 * 1024,
        ),
    )(A_x, A_k_cache, A_v_cache, A_wq, A_wo, B_w_r,
      B_w_gate, B_w_up, B_w_down, c, w_mod)
```

```python
import math

import jax
import jax.numpy as jnp
import jax.experimental.pallas as pl
import jax.experimental.pallas.tpu as pltpu

_S = 2048
_D = 1024
_HQ = 32
_HKV = 4
_DH = 128
_SK = 2048
_W = 512
_F = 3584
_EPS = 1e-5

_REP = _HQ // _HKV
_GW = _REP * _DH
_TM = 512
_NT = _S // _TM
_HP = 2
_NSTEP = _REP // _HP
_RQ = _TM // _NSTEP
_CH = 64
_NMK = 4
_MK = _D // _NMK
_FB = 4
_QSCALE = (_DH ** -0.5) * math.log2(math.e)

_BF = jnp.bfloat16
_F32 = jnp.float32


def _layernorm(x):
    inv_n = 1.0 / x.shape[-1]
    m = jnp.sum(x, axis=-1, keepdims=True) * inv_n
    xc = x - m
    v = jnp.sum(xc * xc, axis=-1, keepdims=True) * inv_n
    return xc * jax.lax.rsqrt(v + _EPS)


def _silu(x):
    return x * jax.nn.sigmoid(x)


def _dot(a, b):
    return jnp.dot(a, b, preferred_element_type=_F32)


def _kernel(
    x_hbm, k_hbm, v_hbm, wq_hbm, wo_hbm, wr_ref, wg_hbm, wu_hbm, wd_hbm, c_ref,
    wmod_hbm,
    out_hbm,
    x_vmem, out_vmem, h2_vmem, k_vmem, v_vmem, wq_vmem, wo_vmem,
    wmod_vmem, wg_vmem, wu_vmem, wd_vmem, h_scr, q_scr,
    x_sem, out_sem, kv_sem, wq_sem, wqp_sem, wo_sem, wmod_sem, ffn_sem, fix_sem,
):
    def x_copy(t):
        rows = pl.ds(t * _TM, _TM)
        return pltpu.make_async_copy(
            x_hbm.at[0, rows, :], x_vmem.at[rows, :], x_sem.at[t])

    def out_copy(t):
        rows = pl.ds(t * _TM, _TM)
        return pltpu.make_async_copy(
            out_vmem.at[rows, :], out_hbm.at[0, rows, :], out_sem.at[t])

    def wmod_a_copy(i):
        rows, cols = pl.ds(i * _MK, _MK), pl.ds(0, 2 * _D)
        return pltpu.make_async_copy(
            wmod_hbm.at[rows, cols], wmod_vmem.at[rows, cols], wmod_sem.at[i])

    def wmod_b_copy(i):
        cols = pl.ds(2 * _D + i * 2 * _D, 2 * _D)
        return pltpu.make_async_copy(
            wmod_hbm.at[:, cols], wmod_vmem.at[:, cols], wmod_sem.at[_NMK + i])

    def wq_copy(g):
        cols = pl.ds(g * _GW, _GW)
        return pltpu.make_async_copy(
            wq_hbm.at[:, cols], wq_vmem.at[:, cols], wq_sem.at[g])

    def wqp_copy(i):
        cols = pl.ds(i * _HP * _DH, _HP * _DH)
        return pltpu.make_async_copy(
            wq_hbm.at[:, cols], wq_vmem.at[:, cols], wqp_sem.at[i])

    def wo_copy(g):
        rows = pl.ds(g * _GW, _GW)
        return pltpu.make_async_copy(
            wo_hbm.at[rows, :], wo_vmem.at[rows, :], wo_sem.at[g])

    window = pl.ds(_SK - _W, _W)
    k_copy = pltpu.make_async_copy(k_hbm.at[0, :, window, :], k_vmem, kv_sem.at[0])
    v_copy = pltpu.make_async_copy(v_hbm.at[0, :, window, :], v_vmem, kv_sem.at[1])
    wg_copy = pltpu.make_async_copy(wg_hbm, wg_vmem, ffn_sem.at[0])
    wu_copy = pltpu.make_async_copy(wu_hbm, wu_vmem, ffn_sem.at[1])
    wd_copy = pltpu.make_async_copy(wd_hbm, wd_vmem, ffn_sem.at[2])

    c = c_ref[...].astype(_F32)
    sc = jnp.broadcast_to(_silu(c), (16, _D)).astype(_BF)
    wr = wr_ref[...].astype(_F32).reshape(1, _D)
    sub_iota = jax.lax.broadcasted_iota(jnp.int32, (8, 1), 0)

    def mod_vector(j):
        return _dot(sc, wmod_vmem[:, j * _D:(j + 1) * _D])[0:1, :]

    def adaln1(t, sa, ca):
        for r0 in range(0, _TM, _CH):
            x = x_vmem[t * _TM + r0:t * _TM + r0 + _CH, :].astype(_F32)
            h_scr[t % 2, r0:r0 + _CH, :] = (_layernorm(x) * ca + sa).astype(_BF)

    def q_piece(slot, g, i):
        c0 = g * _GW + i * _HP * _DH
        return _dot(h_scr[slot], wq_vmem[:, c0:c0 + _HP * _DH]).astype(_BF)

    def o_piece(o, g, i):
        c0 = i * _HP * _DH
        return _dot(o, wo_vmem[g * _GW:(g + 1) * _GW, c0:c0 + _HP * _DH])

    best = [jnp.full((8, 1), -jnp.inf, _F32), jnp.zeros((8, 1), jnp.int32)]

    def epilogue(t, acc, mods):
        ga, sb, cb, gb = mods
        bv, bi = best
        for c0 in range(0, _TM, _CH):
            r0 = t * _TM + c0
            x1 = x_vmem[r0:r0 + _CH, :].astype(_F32) + ga * acc[c0:c0 + _CH, :]
            h2 = _layernorm(x1) * cb + sb
            h2_vmem[r0:r0 + _CH, :] = h2.astype(_BF)
            out_vmem[r0:r0 + _CH, :] = (x1 + gb * h2).astype(_BF)
            r = jnp.sum(h2 * wr, axis=-1, keepdims=True)
            for k in range(0, _CH, 8):
                rk = r[k:k + 8, :]
                gt = rk > bv
                bv = jnp.where(gt, rk, bv)
                bi = jnp.where(gt, sub_iota + (r0 + k), bi)
        best[:] = [bv, bi]

    def step(q, g, i, slot, g_next, o_prev, g_prev, acc):
        scores = [
            jax.lax.dot_general(
                q[:, j * _DH:(j + 1) * _DH], k_vmem[g], (((1,), (1,)), ((), ())),
                preferred_element_type=_F32)
            for j in range(i * _HP, (i + 1) * _HP)]
        q_next = None
        if slot is not None and g_next == 0:
            rows = slice(i * _RQ, (i + 1) * _RQ)
            q_scr[rows, :] = _dot(h_scr[slot, rows, :], wq_vmem[:, 0:_GW]).astype(_BF)
        elif slot is not None:
            q_next = q_piece(slot, g_next, i)
        outs = []
        for s in scores:
            m = jnp.max(s, axis=-1, keepdims=True)
            p = jnp.exp2(s - m)
            l = jnp.sum(p, axis=-1, keepdims=True)
            o = _dot(p.astype(_BF), v_vmem[g])
            outs.append((o * pl.reciprocal(l, approx=True)).astype(_BF))
        if o_prev is not None:
            a = o_piece(o_prev, g_prev, i)
            acc = a if acc is None else acc + a
        return q_next, outs, acc

    x_copy(0).start()
    wmod_a_copy(0).start()
    x_copy(0).wait()
    wmod_a_copy(1).start()
    wmod_a_copy(2).start()
    xhat = _layernorm(x_vmem[0:_TM, :].astype(_F32))
    mod_a = None
    for i in range(_NMK):
        wmod_a_copy(i).wait()
        if i == 0:
            wmod_a_copy(3).start()
        elif i == 2:
            wqp_copy(0).start()
        elif i == 3:
            wqp_copy(1).start()
            wqp_copy(2).start()
        ks = slice(i * _MK, (i + 1) * _MK)
        part = _dot(sc[:, ks], wmod_vmem[ks, 0:2 * _D])
        mod_a = part if mod_a is None else mod_a + part
    sa = mod_a[0:1, 0:_D] * _QSCALE
    ca = (1.0 + mod_a[0:1, _D:2 * _D]) * _QSCALE
    h_scr[0] = (xhat * ca + sa).astype(_BF)
    q_parts = []
    for i in range(_NSTEP):
        wqp_copy(i).wait()
        if i == 0:
            wqp_copy(3).start()
            k_copy.start()
            v_copy.start()
        elif i == 1:
            wq_copy(1).start()
        elif i == 3:
            wo_copy(0).start()
            x_copy(1).start()
            wq_copy(2).start()
        q_parts.append(q_piece(0, 0, i))
    q = jnp.concatenate(q_parts, axis=1)
    k_copy.wait()
    v_copy.wait()

    n_groups = _NT * _HKV
    mods = None
    slot = 0
    acc = [None] * _NSTEP
    acc_done = None
    o_prev = None
    for n in range(n_groups):
        t, g = divmod(n, _HKV)
        t_next, g_next = divmod(n + 1, _HKV)
        g_prev = (n - 1) % _HKV
        if n == 0:
            wq_copy(1).wait()
            wo_copy(1).start()
        elif n == 1:
            wo_copy(0).wait()
            wq_copy(2).wait()
            wq_copy(3).start()
            wo_copy(2).start()
            wo_copy(3).start()
        elif n == 2:
            wo_copy(1).wait()
            wq_copy(3).wait()
            wo_copy(2).wait()
            wo_copy(3).wait()
            wmod_b_copy(0).start()
            wmod_b_copy(1).start()
            for tt in range(2, _NT):
                x_copy(tt).start()
        elif n == 4:
            wg_copy.start()
            wu_copy.start()
            wd_copy.start()
        elif n == 5:
            wmod_b_copy(0).wait()
            wmod_b_copy(1).wait()
            mods = (mod_vector(2), mod_vector(3), 1.0 + mod_vector(4), mod_vector(5))
        if g == 1:
            if t + 1 < _NT:
                x_copy(t + 1).wait()
            if t >= 1:
                epilogue(t - 1, acc_done, mods)
        if g == 2 and t + 1 < _NT:
            adaln1(t + 1, sa, ca)
        if g == 3 and t >= 1:
            out_copy(t - 1).start()

        has_next = t_next < _NT
        if g_next == 0 and has_next:
            slot = t_next % 2
        if g_prev == 0:
            acc = [None] * _NSTEP
        q_next, outs = [], []
        for i in range(_NSTEP):
            qn, o_i, acc[i] = step(q, g, i, slot if has_next else None, g_next,
                                   o_prev, g_prev, acc[i])
            q_next.append(qn)
            outs.extend(o_i)
        if g_prev == _HKV - 1 and n >= 1:
            acc_done = jnp.concatenate(acc, axis=1)
        o_prev = jnp.concatenate(outs, axis=1)
        if has_next:
            q = q_scr[...] if g_next == 0 else jnp.concatenate(q_next, axis=1)
    acc = [acc[i] + o_piece(o_prev, _HKV - 1, i) for i in range(_NSTEP)]
    epilogue(_NT - 1, jnp.concatenate(acc, axis=1), mods)
    out_copy(_NT - 1).start()

    bv, bi = best
    best_r = jnp.max(bv)
    idx = jnp.clip(jnp.min(jnp.where(bv == best_r, bi, _S)), 0, _S - 1)
    base = pl.multiple_of((idx // 16) * 16, 16)
    rows = pl.ds(base, 16)
    sel = jax.lax.broadcasted_iota(jnp.int32, (16, 1), 0) == (idx - base)
    h2blk = h2_vmem[rows, :]
    wg_copy.wait()
    wu_copy.wait()
    wd_copy.wait()
    y = None
    fb = _F // _FB
    for i in range(_FB):
        fs = slice(i * fb, (i + 1) * fb)
        gate = _dot(h2blk, wg_vmem[:, fs])
        up = _dot(h2blk, wu_vmem[:, fs])
        part = _dot((_silu(gate) * up).astype(_BF), wd_vmem[fs, :])
        y = part if y is None else y + part
    y = y * jax.nn.sigmoid(jnp.full((1, _D), best_r, _F32))
    for t in range(_NT):
        out_copy(t).wait()
    blk = out_vmem[rows, :].astype(_F32)
    out_vmem[rows, :] = jnp.where(sel, blk + mods[3] * y, blk).astype(_BF)
    fix = pltpu.make_async_copy(out_vmem.at[rows, :], out_hbm.at[0, rows, :], fix_sem)
    fix.start()
    fix.wait()


@jax.jit
def pallas_adaLN_cond__sliding_block_cached__moe_arch_mod__prompt_kernel(
    A_x: jax.Array,
    A_k_cache: jax.Array,
    A_v_cache: jax.Array,
    A_wq: jax.Array,
    A_wo: jax.Array,
    B_x: jax.Array,
    B_w_r: jax.Array,
    B_w_gate: jax.Array,
    B_w_up: jax.Array,
    B_w_down: jax.Array,
    c: jax.Array,
    w_mod: jax.Array,
):
    del B_x
    any_spec = pl.BlockSpec(memory_space=pl.ANY)
    vmem_spec = pl.BlockSpec(memory_space=pltpu.VMEM)
    dma = pltpu.SemaphoreType.DMA
    return pl.pallas_call(
        _kernel,
        out_shape=jax.ShapeDtypeStruct(A_x.shape, A_x.dtype),
        in_specs=[
            any_spec, any_spec, any_spec, any_spec, any_spec,
            vmem_spec,
            any_spec, any_spec, any_spec,
            vmem_spec,
            any_spec,
        ],
        out_specs=any_spec,
        scratch_shapes=[
            pltpu.VMEM((_S, _D), _BF),
            pltpu.VMEM((_S, _D), _BF),
            pltpu.VMEM((_S, _D), _BF),
            pltpu.VMEM((_HKV, _W, _DH), _BF),
            pltpu.VMEM((_HKV, _W, _DH), _BF),
            pltpu.VMEM((_D, _HQ * _DH), _BF),
            pltpu.VMEM((_HQ * _DH, _D), _BF),
            pltpu.VMEM((_D, 6 * _D), _BF),
            pltpu.VMEM((_D, _F), _BF),
            pltpu.VMEM((_D, _F), _BF),
            pltpu.VMEM((_F, _D), _BF),
            pltpu.VMEM((2, _TM, _D), _BF),
            pltpu.VMEM((_TM, _GW), _BF),
            dma((_NT,)),
            dma((_NT,)),
            dma((2,)),
            dma((_HKV,)),
            dma((_NSTEP,)),
            dma((_HKV,)),
            dma((_NMK + 2,)),
            dma((3,)),
            dma(()),
        ],
        compiler_params=pltpu.CompilerParams(
            vmem_limit_bytes=110 * 1024 * 1024,
        ),
    )(A_x, A_k_cache, A_v_cache, A_wq, A_wo, B_w_r,
      B_w_gate, B_w_up, B_w_down, c, w_mod)
```

```python
import math

import jax
import jax.numpy as jnp
import jax.experimental.pallas as pl
import jax.experimental.pallas.tpu as pltpu

_S = 2048
_D = 1024
_HQ = 32
_HKV = 4
_DH = 128
_SK = 2048
_W = 512
_F = 3584
_EPS = 1e-5

_REP = _HQ // _HKV
_GW = _REP * _DH
_TM = 512
_NT = _S // _TM
_HP = 2
_NSTEP = _REP // _HP
_RQ = _TM // _NSTEP
_CH = 64
_NMK = 4
_MK = _D // _NMK
_FB = 4
_QSCALE = (_DH ** -0.5) * math.log2(math.e)

_BF = jnp.bfloat16
_F32 = jnp.float32


def _layernorm(x):
    inv_n = 1.0 / x.shape[-1]
    m = jnp.sum(x, axis=-1, keepdims=True) * inv_n
    xc = x - m
    v = jnp.sum(xc * xc, axis=-1, keepdims=True) * inv_n
    return xc * jax.lax.rsqrt(v + _EPS)


def _silu(x):
    return x * jax.nn.sigmoid(x)


def _dot(a, b):
    return jnp.dot(a, b, preferred_element_type=_F32)


def _kernel(
    x_hbm, k_hbm, v_hbm, wq_hbm, wo_hbm, wr_hbm, wg_hbm, wu_hbm, wd_hbm, c_hbm,
    wmod_hbm,
    out_hbm,
    x_vmem, out_vmem, h2_vmem, k_vmem, v_vmem, wq_vmem, wo_vmem,
    wmod_vmem, wg_vmem, wu_vmem, wd_vmem, h_scr, q_scr, c_vmem, wr_vmem,
    x_sem, out_sem, kv_sem, wq_sem, wqp_sem, wo_sem, wmod_sem, ffn_sem, fix_sem,
):
    def x_copy(t):
        rows = pl.ds(t * _TM, _TM)
        return pltpu.make_async_copy(
            x_hbm.at[0, rows, :], x_vmem.at[rows, :], x_sem.at[t])

    def out_copy(t):
        rows = pl.ds(t * _TM, _TM)
        return pltpu.make_async_copy(
            out_vmem.at[rows, :], out_hbm.at[0, rows, :], out_sem.at[t])

    def wmod_a_copy(i):
        rows, cols = pl.ds(i * _MK, _MK), pl.ds(0, 2 * _D)
        return pltpu.make_async_copy(
            wmod_hbm.at[rows, cols], wmod_vmem.at[rows, cols], wmod_sem.at[i])

    def wmod_b_copy(i):
        cols = pl.ds(2 * _D + i * 2 * _D, 2 * _D)
        return pltpu.make_async_copy(
            wmod_hbm.at[:, cols], wmod_vmem.at[:, cols], wmod_sem.at[_NMK + i])

    def wq_copy(g):
        cols = pl.ds(g * _GW, _GW)
        return pltpu.make_async_copy(
            wq_hbm.at[:, cols], wq_vmem.at[:, cols], wq_sem.at[g])

    def wqp_copy(i):
        cols = pl.ds(i * _HP * _DH, _HP * _DH)
        return pltpu.make_async_copy(
            wq_hbm.at[:, cols], wq_vmem.at[:, cols], wqp_sem.at[i])

    def wo_copy(g):
        rows = pl.ds(g * _GW, _GW)
        return pltpu.make_async_copy(
            wo_hbm.at[rows, :], wo_vmem.at[rows, :], wo_sem.at[g])

    window = pl.ds(_SK - _W, _W)
    k_copy = pltpu.make_async_copy(k_hbm.at[0, :, window, :], k_vmem, kv_sem.at[0])
    v_copy = pltpu.make_async_copy(v_hbm.at[0, :, window, :], v_vmem, kv_sem.at[1])
    wg_copy = pltpu.make_async_copy(wg_hbm, wg_vmem, ffn_sem.at[0])
    wu_copy = pltpu.make_async_copy(wu_hbm, wu_vmem, ffn_sem.at[1])
    wd_copy = pltpu.make_async_copy(wd_hbm, wd_vmem, ffn_sem.at[2])

    c_copy = pltpu.make_async_copy(c_hbm, c_vmem, kv_sem.at[2])
    wr_copy = pltpu.make_async_copy(wr_hbm, wr_vmem, kv_sem.at[3])
    x_copy(0).start()
    wmod_a_copy(0).start()
    c_copy.start()
    wr_copy.start()
    c_copy.wait()

    c = c_vmem[...].astype(_F32)
    sc = jnp.broadcast_to(_silu(c), (16, _D)).astype(_BF)
    small = {}
    sub_iota = jax.lax.broadcasted_iota(jnp.int32, (8, 1), 0)

    def mod_vector(j):
        return _dot(sc, wmod_vmem[:, j * _D:(j + 1) * _D])[0:1, :]

    def adaln1(t, sa, ca):
        for r0 in range(0, _TM, _CH):
            x = x_vmem[t * _TM + r0:t * _TM + r0 + _CH, :].astype(_F32)
            h_scr[t % 2, r0:r0 + _CH, :] = (_layernorm(x) * ca + sa).astype(_BF)

    def q_piece(slot, g, i):
        c0 = g * _GW + i * _HP * _DH
        return _dot(h_scr[slot], wq_vmem[:, c0:c0 + _HP * _DH]).astype(_BF)

    def o_piece(o, g, i):
        c0 = i * _HP * _DH
        return _dot(o, wo_vmem[g * _GW:(g + 1) * _GW, c0:c0 + _HP * _DH])

    best = [jnp.full((8, 1), -jnp.inf, _F32), jnp.zeros((8, 1), jnp.int32)]

    def epilogue(t, acc, mods):
        ga, sb, cb, gb = mods
        bv, bi = best
        for c0 in range(0, _TM, _CH):
            r0 = t * _TM + c0
            x1 = x_vmem[r0:r0 + _CH, :].astype(_F32) + ga * acc[c0:c0 + _CH, :]
            h2 = _layernorm(x1) * cb + sb
            h2_vmem[r0:r0 + _CH, :] = h2.astype(_BF)
            out_vmem[r0:r0 + _CH, :] = (x1 + gb * h2).astype(_BF)
            r = jnp.sum(h2 * small["wr"], axis=-1, keepdims=True)
            for k in range(0, _CH, 8):
                rk = r[k:k + 8, :]
                gt = rk > bv
                bv = jnp.where(gt, rk, bv)
                bi = jnp.where(gt, sub_iota + (r0 + k), bi)
        best[:] = [bv, bi]

    def step(q, g, i, slot, g_next, o_prev, g_prev, acc):
        scores = [
            jax.lax.dot_general(
                q[:, j * _DH:(j + 1) * _DH], k_vmem[g], (((1,), (1,)), ((), ())),
                preferred_element_type=_F32)
            for j in range(i * _HP, (i + 1) * _HP)]
        q_next = None
        if slot is not None and g_next == 0:
            rows = slice(i * _RQ, (i + 1) * _RQ)
            q_scr[rows, :] = _dot(h_scr[slot, rows, :], wq_vmem[:, 0:_GW]).astype(_BF)
        elif slot is not None:
            q_next = q_piece(slot, g_next, i)
        outs = []
        for s in scores:
            m = jnp.max(s, axis=-1, keepdims=True)
            p = jnp.exp2(s - m)
            l = jnp.sum(p, axis=-1, keepdims=True)
            o = _dot(p.astype(_BF), v_vmem[g])
            outs.append((o * pl.reciprocal(l, approx=True)).astype(_BF))
        if o_prev is not None:
            a = o_piece(o_prev, g_prev, i)
            acc = a if acc is None else acc + a
        return q_next, outs, acc

    x_copy(0).wait()
    wmod_a_copy(1).start()
    wmod_a_copy(2).start()
    xhat = _layernorm(x_vmem[0:_TM, :].astype(_F32))
    mod_a = None
    for i in range(_NMK):
        wmod_a_copy(i).wait()
        if i == 0:
            wmod_a_copy(3).start()
        elif i == 2:
            wqp_copy(0).start()
        elif i == 3:
            wqp_copy(1).start()
            wqp_copy(2).start()
        ks = slice(i * _MK, (i + 1) * _MK)
        part = _dot(sc[:, ks], wmod_vmem[ks, 0:2 * _D])
        mod_a = part if mod_a is None else mod_a + part
    sa = mod_a[0:1, 0:_D] * _QSCALE
    ca = (1.0 + mod_a[0:1, _D:2 * _D]) * _QSCALE
    h_scr[0] = (xhat * ca + sa).astype(_BF)
    q_parts = []
    for i in range(_NSTEP):
        wqp_copy(i).wait()
        if i == 0:
            wqp_copy(3).start()
            k_copy.start()
            v_copy.start()
        elif i == 1:
            wq_copy(1).start()
        elif i == 3:
            wo_copy(0).start()
            x_copy(1).start()
            wq_copy(2).start()
        q_parts.append(q_piece(0, 0, i))
    q = jnp.concatenate(q_parts, axis=1)
    k_copy.wait()
    v_copy.wait()

    n_groups = _NT * _HKV
    mods = None
    slot = 0
    acc = [None] * _NSTEP
    acc_done = None
    o_prev = None
    for n in range(n_groups):
        t, g = divmod(n, _HKV)
        t_next, g_next = divmod(n + 1, _HKV)
        g_prev = (n - 1) % _HKV
        if n == 0:
            wq_copy(1).wait()
            wo_copy(1).start()
        elif n == 1:
            wr_copy.wait()
            small["wr"] = wr_vmem[...].astype(_F32).reshape(1, _D)
            wo_copy(0).wait()
            wq_copy(2).wait()
            wq_copy(3).start()
            wo_copy(2).start()
            wo_copy(3).start()
        elif n == 2:
            wo_copy(1).wait()
            wq_copy(3).wait()
            wo_copy(2).wait()
            wo_copy(3).wait()
            wmod_b_copy(0).start()
            wmod_b_copy(1).start()
            for tt in range(2, _NT):
                x_copy(tt).start()
        elif n == 4:
            wg_copy.start()
            wu_copy.start()
            wd_copy.start()
        elif n == 5:
            wmod_b_copy(0).wait()
            wmod_b_copy(1).wait()
            mods = (mod_vector(2), mod_vector(3), 1.0 + mod_vector(4), mod_vector(5))
        if g == 1:
            if t + 1 < _NT:
                x_copy(t + 1).wait()
            if t >= 1:
                epilogue(t - 1, acc_done, mods)
        if g == 2 and t + 1 < _NT:
            adaln1(t + 1, sa, ca)
        if g == 3 and t >= 1:
            out_copy(t - 1).start()

        has_next = t_next < _NT
        if g_next == 0 and has_next:
            slot = t_next % 2
        if g_prev == 0:
            acc = [None] * _NSTEP
        q_next, outs = [], []
        for i in range(_NSTEP):
            qn, o_i, acc[i] = step(q, g, i, slot if has_next else None, g_next,
                                   o_prev, g_prev, acc[i])
            q_next.append(qn)
            outs.extend(o_i)
        if g_prev == _HKV - 1 and n >= 1:
            acc_done = jnp.concatenate(acc, axis=1)
        o_prev = jnp.concatenate(outs, axis=1)
        if has_next:
            q = q_scr[...] if g_next == 0 else jnp.concatenate(q_next, axis=1)
    acc = [acc[i] + o_piece(o_prev, _HKV - 1, i) for i in range(_NSTEP)]
    epilogue(_NT - 1, jnp.concatenate(acc, axis=1), mods)
    out_copy(_NT - 1).start()

    bv, bi = best
    best_r = jnp.max(bv)
    idx = jnp.clip(jnp.min(jnp.where(bv == best_r, bi, _S)), 0, _S - 1)
    base = pl.multiple_of((idx // 16) * 16, 16)
    rows = pl.ds(base, 16)
    sel = jax.lax.broadcasted_iota(jnp.int32, (16, 1), 0) == (idx - base)
    h2blk = h2_vmem[rows, :]
    wg_copy.wait()
    wu_copy.wait()
    wd_copy.wait()
    y = None
    fb = _F // _FB
    for i in range(_FB):
        fs = slice(i * fb, (i + 1) * fb)
        gate = _dot(h2blk, wg_vmem[:, fs])
        up = _dot(h2blk, wu_vmem[:, fs])
        part = _dot((_silu(gate) * up).astype(_BF), wd_vmem[fs, :])
        y = part if y is None else y + part
    y = y * jax.nn.sigmoid(jnp.full((1, _D), best_r, _F32))
    for t in range(_NT):
        out_copy(t).wait()
    blk = out_vmem[rows, :].astype(_F32)
    out_vmem[rows, :] = jnp.where(sel, blk + mods[3] * y, blk).astype(_BF)
    fix = pltpu.make_async_copy(out_vmem.at[rows, :], out_hbm.at[0, rows, :], fix_sem)
    fix.start()
    fix.wait()


@jax.jit
def pallas_adaLN_cond__sliding_block_cached__moe_arch_mod__prompt_kernel(
    A_x: jax.Array,
    A_k_cache: jax.Array,
    A_v_cache: jax.Array,
    A_wq: jax.Array,
    A_wo: jax.Array,
    B_x: jax.Array,
    B_w_r: jax.Array,
    B_w_gate: jax.Array,
    B_w_up: jax.Array,
    B_w_down: jax.Array,
    c: jax.Array,
    w_mod: jax.Array,
):
    del B_x
    any_spec = pl.BlockSpec(memory_space=pl.ANY)
    dma = pltpu.SemaphoreType.DMA
    return pl.pallas_call(
        _kernel,
        out_shape=jax.ShapeDtypeStruct(A_x.shape, A_x.dtype),
        in_specs=[
            any_spec, any_spec, any_spec, any_spec, any_spec,
            any_spec,
            any_spec, any_spec, any_spec,
            any_spec,
            any_spec,
        ],
        out_specs=any_spec,
        scratch_shapes=[
            pltpu.VMEM((_S, _D), _BF),
            pltpu.VMEM((_S, _D), _BF),
            pltpu.VMEM((_S, _D), _BF),
            pltpu.VMEM((_HKV, _W, _DH), _BF),
            pltpu.VMEM((_HKV, _W, _DH), _BF),
            pltpu.VMEM((_D, _HQ * _DH), _BF),
            pltpu.VMEM((_HQ * _DH, _D), _BF),
            pltpu.VMEM((_D, 6 * _D), _BF),
            pltpu.VMEM((_D, _F), _BF),
            pltpu.VMEM((_D, _F), _BF),
            pltpu.VMEM((_F, _D), _BF),
            pltpu.VMEM((2, _TM, _D), _BF),
            pltpu.VMEM((_TM, _GW), _BF),
            pltpu.VMEM((1, _D), _BF),
            pltpu.VMEM((_D,), _BF),
            dma((_NT,)),
            dma((_NT,)),
            dma((4,)),
            dma((_HKV,)),
            dma((_NSTEP,)),
            dma((_HKV,)),
            dma((_NMK + 2,)),
            dma((3,)),
            dma(()),
        ],
        compiler_params=pltpu.CompilerParams(
            vmem_limit_bytes=110 * 1024 * 1024,
        ),
    )(A_x, A_k_cache, A_v_cache, A_wq, A_wo, B_w_r,
      B_w_gate, B_w_up, B_w_down, c, w_mod)
```
